```python
import os as _os
_os.environ.setdefault("JAX_PLATFORMS", "cpu")
import jax
import jax.numpy as jnp

def _softmax(x, axis=-1):
    return jax.nn.softmax(x, axis=axis)
def _gelu(x):
    return jax.nn.gelu(x, approximate=True)
def _silu(x):
    return jax.nn.silu(x)
def _sigmoid(x):
    return jax.nn.sigmoid(x)
def _layernorm(x, axis=-1, eps=1e-5):
    m = jnp.mean(x, axis=axis, keepdims=True)
    v = jnp.var(x, axis=axis, keepdims=True)
    return (x - m) / jnp.sqrt(v + eps)
def _scatter_add(tgt, idx, src, axis=0):
    return tgt.at[idx].add(src)
def _segment_sum(src, seg, n):
    return jax.ops.segment_sum(src, seg, n)
class _Rng:
    def __init__(self, key):
        self._k = key
    def _next(self):
        self._k, sub = jax.random.split(self._k)
        return sub
    def normal(self, shape):
        return jax.random.normal(self._next(), shape, dtype=jnp.bfloat16)
    def randint(self, lo, hi, shape):
        return jax.random.randint(self._next(), shape, lo, hi, dtype=jnp.int32)
    def uniform(self, shape, lo=0.0, hi=1.0):
        return jax.random.uniform(self._next(), shape, jnp.bfloat16, lo, hi)
    def permutation(self, n):
        return jax.random.permutation(self._next(), n)


kernel_name = 'interleave_layers__spectral_gfnet__dense_activation_gelu__prompt'

def setup_inputs():
    _rng = _Rng(jax.random.key(int.from_bytes(__import__("os").urandom(4), "little")))
    _w = (lambda a: (lambda t: t.astype(jnp.bfloat16) if jnp.issubdtype(t.dtype, jnp.floating) else t)(jnp.asarray(a)))
    def _A_setup():
        B, S, D = 1, 2048, 640
        Df = D // 2 + 1
        return {
            "x": _w((lambda *s: _rng.normal(s) * 0.05)(B, S, D)),
            "w_r": _w((lambda *s: _rng.normal(s) * 0.2)(S, Df) * 0.02),
            "w_i": _w((lambda *s: _rng.normal(s) * 0.2)(S, Df) * 0.02),
        }
    _A_in = _A_setup()

    def _B_setup():
        B, S, D, F = 1, 2048, 640, 1728
        return {
            "x": _w((lambda *s: _rng.normal(s) * 0.05)(B, S, D)),
            "w1": _w((lambda *s: _rng.normal(s) * 0.1)(D, F) * (D ** -0.5)),
            "b1": _w((lambda *s: _rng.normal(s) * 0.1)(F) * 0.01),
            "w2": _w((lambda *s: _rng.normal(s) * 0.1)(F, D) * (F ** -0.5)),
            "b2": _w((lambda *s: _rng.normal(s) * 0.1)(D) * 0.01),
        }
    _B_in = _B_setup()

    return {
        "A_x": _A_in["x"],
        "A_w_r": _A_in["w_r"],
        "A_w_i": _A_in["w_i"],
        "B_x": _B_in["x"],
        "B_w1": _B_in["w1"],
        "B_b1": _B_in["b1"],
        "B_w2": _B_in["w2"],
        "B_b2": _B_in["b2"],
    }

def reference(A_x, A_w_r, A_w_i, B_x, B_w1, B_b1, B_w2, B_b2):
    def _A_ref(x, w_r, w_i):
        B, S, D = x.shape
        X = (lambda x, axes=(-2,-1): jnp.fft.rfft2(x.astype(jnp.float32), axes=axes))(x, axes=(-2, -1))
        W = w_r + 1j * w_i
        X = X * W
        y = (lambda x, s, axes=(-2,-1): jnp.fft.irfft2(x, s=s, axes=axes).astype(jnp.bfloat16))(X, (S, D), axes=(-2, -1))
        return y

    def _B_ref(x, w1, b1, w2, b2):
        h = jnp.einsum("bsd,df->bsf", x, w1) + b1
        h = _gelu(h)
        return jnp.einsum("bsf,fd->bsd", h, w2) + b2

    x = A_x
    x = x + _A_ref(_layernorm(x, axis=-1), A_w_r, A_w_i)
    x = x + _B_ref(_layernorm(x, axis=-1), B_w1, B_b1, B_w2, B_b2)
    x = x + _A_ref(_layernorm(x, axis=-1), A_w_r, A_w_i)
    x = x + _B_ref(_layernorm(x, axis=-1), B_w1, B_b1, B_w2, B_b2)
    return x
```

```python
import functools
import math

import jax
import jax.numpy as jnp
import numpy as np
import jax.experimental.pallas as pl
import jax.experimental.pallas.tpu as pltpu

S, D, F = 2048, 640, 1728
NK = D // 2 + 1
NB, NL = 32, 64
NT = 8
R = S // NT
LANES = 128
EPS = 1e-5
JORD = [k + d for k in range(8) for d in (0, 16, 8, 24)]
JPOS = [JORD.index(j) for j in range(NB)]
F32, BF16 = jnp.float32, jnp.bfloat16


def _lane_layout():
    grp = lambda k: 0 if k % 5 in (1, 4) else (1 if k % 5 in (2, 3) else 2)
    pools = [[[k for k in range(NK) if k // LANES == s and grp(k) == g] for g in range(3)]
             for s in range(3)]
    n = [[len(p) for p in row] for row in pools]
    types = {"A": (0, 1, 2), "B": (1, 0, 2), "C": (0, 2, 1),
             "D": (2, 0, 1), "E": (1, 2, 0), "F": (2, 1, 0)}
    for c in range(LANES + 1):
        cnt = {"C": c, "D": n[1][2] - c}
        cnt["F"] = n[2][0] - cnt["D"]
        cnt["E"] = n[0][2] - cnt["F"]
        cnt["A"] = n[0][0] - cnt["C"]
        cnt["B"] = n[0][1] - cnt["D"]
        if (min(cnt.values()) >= 0 and sum(cnt.values()) == LANES
                and cnt["C"] + cnt["E"] == n[2][1] and cnt["B"] + cnt["E"] == n[1][0]
                and cnt["A"] + cnt["F"] == n[1][1] and cnt["A"] + cnt["B"] >= n[2][2]):
            break
    else:
        raise AssertionError("no lane layout")
    kd = -np.ones((3, LANES), np.int64)
    src = np.zeros((3, LANES), np.int32)
    idx = np.zeros((3, LANES), np.int32)
    p = 0
    for name in "ABCDEF":
        for _ in range(cnt[name]):
            for g, s in enumerate(types[name]):
                if pools[s][g]:
                    k = pools[s][g].pop(0)
                    kd[g, p], src[g, p], idx[s, p] = k, s, k % LANES
            p += 1
    assert p == LANES and not any(q for row in pools for q in row)
    return kd, src, idx


def _d_tables(kd):
    ld = np.arange(LANES)
    fwd, inv = [], []
    for g in range(3):
        k = kd[g]
        used = k >= 0
        th = 2 * np.pi * np.outer(ld, np.where(used, k, 0)) / D
        c, s = np.cos(th) * used, np.sin(th) * used
        if g < 2:
            neg = np.isin(k % 5, (3, 4))
            sg = np.where(neg, -1.0, 1.0)[None, :]
            fwd += [c, -s, s * sg, c * sg]
            w = 2.0 / D
            sgi = np.where(neg, -1.0, 1.0)[:, None]
            inv += [c.T * w, s.T * w * sgi, -s.T * w, c.T * w * sgi]
        else:
            fwd += [c, -s]
            w = np.where((k == 0) | (k == NK - 1), 1.0, 2.0)[:, None] / D
            inv += [c.T * w, -s.T * w]
    return np.stack(fwd + inv + [np.eye(LANES)])


def _s_tables():
    a = np.arange(NL)[:, None]
    l = np.arange(NL)[None, :]
    kap = 16 * (np.arange(NL) // 8) + np.arange(NL) % 8
    mf = np.zeros((NB, 128, 128))
    for b in range(NB):
        m = np.exp(-2j * np.pi * l * (NB * a + b) / S)
        mf[b][np.ix_(np.arange(NL), kap)] = m.real
        mf[b][np.ix_(np.arange(NL), kap + 8)] = -m.imag
        mf[b][np.ix_(NL + np.arange(NL), kap)] = m.imag
        mf[b][np.ix_(NL + np.arange(NL), kap + 8)] = m.real
    mi = np.transpose(mf, (0, 2, 1)) / S
    return mf, mi


_KD, _SRC, _IDX = _lane_layout()
_DM = _d_tables(_KD)
_MF, _MI = _s_tables()
_GT = np.concatenate([np.broadcast_to(_IDX[:, None, :], (3, 8, LANES)),
                      np.broadcast_to(_SRC[:, None, :], (3, 8, LANES))]).astype(np.int32)

C1, S1 = math.cos(2 * math.pi / 5), math.sin(2 * math.pi / 5)
C2, S2 = math.cos(4 * math.pi / 5), math.sin(4 * math.pi / 5)


def _fft(xr, xi, sign):
    n = len(xr)
    if n == 1:
        return list(xr), list(xi)
    if n == 2:
        return [xr[0] + xr[1], xr[0] - xr[1]], [xi[0] + xi[1], xi[0] - xi[1]]
    ur, ui = _fft(xr[0::2], xi[0::2], sign)
    zr, zi = _fft(xr[1::4], xi[1::4], sign)
    wr, wi = _fft(xr[3::4], xi[3::4], sign)
    q = n // 4
    outr, outi = [None] * n, [None] * n

    def twiddle(r, i, k):
        k %= n
        if k == 0:
            return r, i
        if 8 * k == n:
            h = math.sqrt(0.5)
            return ((r - i) * h, (r + i) * h) if sign > 0 else ((r + i) * h, (i - r) * h)
        if 8 * k == 3 * n:
            h = math.sqrt(0.5)
            return ((r + i) * -h, (r - i) * h) if sign > 0 else ((i - r) * h, (r + i) * -h)
        c, s = math.cos(2 * math.pi * k / n), sign * math.sin(2 * math.pi * k / n)
        return r * c - i * s, r * s + i * c

    for k in range(q):
        ar, ai = twiddle(zr[k], zi[k], k)
        br, bi = twiddle(wr[k], wi[k], 3 * k)
        sr, si, dr, di = ar + br, ai + bi, ar - br, ai - bi
        outr[k], outi[k] = ur[k] + sr, ui[k] + si
        outr[k + 2 * q], outi[k + 2 * q] = ur[k] - sr, ui[k] - si
        if sign > 0:
            outr[k + q], outi[k + q] = ur[k + q] - di, ui[k + q] + dr
            outr[k + 3 * q], outi[k + 3 * q] = ur[k + q] + di, ui[k + q] - dr
        else:
            outr[k + q], outi[k + q] = ur[k + q] + di, ui[k + q] - dr
            outr[k + 3 * q], outi[k + 3 * q] = ur[k + q] - di, ui[k + q] + dr
    return outr, outi


def _tiles(x):
    return [x[:, LANES * c:LANES * (c + 1)] for c in range(x.shape[1] // LANES)]


def _layernorm(x):
    m = jnp.mean(x, axis=-1, keepdims=True)
    xc = x - m
    v = jnp.mean(xc * xc, axis=-1, keepdims=True)
    return xc * jax.lax.rsqrt(v + EPS)


def _radix5_fwd(z):
    z0, z1, z2, z3, z4 = _tiles(z)
    a, b, c, e = z1 + z4, z2 + z3, z1 - z4, z2 - z3
    p = a + b
    base = z0 + p * -0.25
    m2 = (a - b) * (math.sqrt(5.0) / 4)
    return [base + m2, c * -S1 + e * -S2, base - m2, e * S1 - c * S2, z0 + p]


def _radix5_inv(a1, b1, a2, b2, s0):
    p = a1 + a2
    base = s0 + p * -0.25
    m2 = (a1 - a2) * (math.sqrt(5.0) / 4)
    e1, e2 = base + m2, base - m2
    o1 = b1 * S1 + b2 * S2
    o2 = b1 * S2 - b2 * S1
    return jnp.concatenate([s0 + p, e1 - o1, e2 - o2, e2 + o2, e1 + o1], axis=1)


def _gelu(h):
    c = math.sqrt(2.0 / math.pi)
    u = h * (c + (c * 0.044715) * (h * h))
    hh = 0.5 * h
    return hh + hh * jnp.tanh(u)


def _dot(a, b):
    return jnp.dot(a, b, preferred_element_type=F32)


def _block(ref, i0, nr, nc):
    return jnp.concatenate(
        [jnp.concatenate([ref[i0 + r * nc + c] for c in range(nc)], axis=1) for r in range(nr)],
        axis=0)


SEM_X, SEM_O, SEM_W1, SEM_W2, SEM_T, SEM_W = 0, 8, 16, 21, 26, 32
N_SEM = 64
PITCH = NL + 1


def _kernel(x_hbm, wr_hbm, wi_hbm, w1_hbm, b1_hbm, w2_hbm, b2_hbm, dm_hbm, mf_hbm, mi_hbm, gt_hbm,
            out_hbm,
            xs, x2s, outs, ws, wp, w1s, w2s, b1s, b2s, b1f, b2f, dms, mfs, mis, gts,
            ub, yb, vb, tb, z1b, x1b, hb, sems):

    def x_copy(t):
        return pltpu.make_async_copy(x_hbm.at[:, t], xs.at[t], sems.at[SEM_X + t])

    def o_copy(t):
        return pltpu.make_async_copy(outs.at[t], out_hbm.at[:, t], sems.at[SEM_O + t])

    w_copies = [[pltpu.make_async_copy(w_hbm.at[:, LANES * q:LANES * (q + 1)], ws.at[a, q],
                                       sems.at[SEM_W + 16 * a + q]) for q in range(16)]
                for a, w_hbm in enumerate((wr_hbm, wi_hbm))]
    w1_copies = [pltpu.make_async_copy(w1_hbm.at[:, LANES * c:LANES * (c + 1)], w1s.at[c],
                                       sems.at[SEM_W1 + c]) for c in range(5)]
    w2_copies = [pltpu.make_async_copy(w2_hbm.at[:, LANES * c:LANES * (c + 1)], w2s.at[c],
                                       sems.at[SEM_W2 + c]) for c in range(5)]
    t_copies = [pltpu.make_async_copy(s, d, sems.at[SEM_T + i]) for i, (s, d) in enumerate(
        ((dm_hbm, dms), (gt_hbm, gts), (mf_hbm, mfs), (mi_hbm, mis), (b1_hbm, b1s), (b2_hbm, b2s)))]

    x_copy(0).start()
    t_copies[0].start()
    for t in range(1, NT):
        x_copy(t).start()
    t_copies[1].start()
    for c in w_copies[0] + w_copies[1]:
        c.start()
    for c in t_copies[2:]:
        c.start()
    for c in w1_copies + w2_copies:
        c.start()

    val = {}

    def load_x(t):
        return jnp.concatenate([xs[t, j].astype(F32) for j in JORD], axis=0)

    def put_t(t, z):
        for c, v in enumerate(_radix5_fwd(z)):
            tb[t, c] = v.astype(BF16)

    def ln0(t):
        put_t(t, _layernorm(load_x(t)))

    def c_mm(t, g):
        if g < 2:
            x = _dot(jnp.concatenate([tb[t, 2 * g], tb[t, 2 * g + 1]], axis=1),
                     _block(dms, 4 * g, 2, 2))
        else:
            x = _dot(tb[t, 4], _block(dms, 8, 1, 2))
        val["c", t, g] = x

    def c_fft(t, g):
        x = val.pop(("c", t, g))
        ur, ui = _fft([x[8 * JPOS[j]:8 * JPOS[j] + 8, :LANES] for j in range(NB)],
                      [x[8 * JPOS[j]:8 * JPOS[j] + 8, LANES:] for j in range(NB)], -1)
        for b in range(NB):
            ub[b, g, 16 * t:16 * t + 16, :] = jnp.concatenate([ur[b], ui[b]], axis=0).astype(BF16)

    def prep_w(a, q):
        ident = dms[20]
        nt = (((1,), (1,)), ((), ()))
        p = []
        for c in range(3):
            hi = min(LANES * (c + 1), NK)
            wt = jax.lax.dot_general(ident, ws[a, q, LANES * c:hi, :], nt,
                                     preferred_element_type=F32)
            if hi - LANES * c < LANES:
                wt = jnp.pad(wt, ((0, 0), (0, LANES * (c + 1) - hi)))
            wt = pltpu.bitcast(wt.astype(BF16), jnp.uint32)
            p.append(jnp.take_along_axis(
                wt, jnp.broadcast_to(gts[c, 0:1, :], (NL, LANES)), axis=1))
        for g in range(3):
            src = gts[3 + g, 0:1, :]
            w = jnp.where(src == 0, p[0], jnp.where(src == 1, p[1], p[2]))
            for r in range(8):
                wp[a, g, pl.ds(PITCH * 8 * (r % 2) + 4 * q + r // 2, 8, stride=PITCH), :] = (
                    w[8 * r:8 * r + 8])

    def p_fwd(b2, g):
        wg = [wp[a, g, pl.ds(PITCH * b2, NL), :] for a in range(2)]
        for par in range(2):
            b = 2 * b2 + par
            if par == 0:
                wr, wi = [pltpu.bitcast(w << 16, F32) for w in wg]
            else:
                wr, wi = [pltpu.bitcast(w & jnp.uint32(0xFFFF0000), F32) for w in wg]
            xf = _dot(mfs[b], ub[b, g])
            xr, xi = xf[:NL], xf[NL:]
            yb[b, g] = jnp.concatenate([xr * wr - xi * wi, xr * wi + xi * wr], axis=0).astype(BF16)

    def p_inv(b2, g):
        for b in (2 * b2, 2 * b2 + 1):
            vb[b, g] = _dot(mis[b], yb[b, g]).astype(BF16)

    def a_fft(t, g):
        v = [vb[b, g, 16 * t:16 * t + 16, :].astype(F32) for b in range(NB)]
        yr, yi = _fft([q[:8] for q in v], [q[8:] for q in v], +1)
        val["a", t, g] = jnp.concatenate(
            [jnp.concatenate([yr[j] for j in JORD], axis=0).astype(BF16),
             jnp.concatenate([yi[j] for j in JORD], axis=0).astype(BF16)], axis=1)

    def a_mm(t, g):
        y = val.pop(("a", t, g))
        val["s", t, g] = _dot(y, _block(dms, 10 + 4 * g, 2, 2 if g < 2 else 1))

    def a_tail(t, layer):
        s1, s2, s0 = [val.pop(("s", t, g)) for g in range(3)]
        y = _radix5_inv(s1[:, :LANES], s1[:, LANES:], s2[:, :LANES], s2[:, LANES:], s0)
        if layer == 0:
            x0 = load_x(t)
        else:
            x0 = jnp.concatenate([x2s[t, c].astype(F32) for c in range(5)], axis=1)
        x1 = x0 + y
        x1b[t] = x1
        for c, zc in enumerate(_tiles(_layernorm(x1))):
            z1b[t, c] = zc.astype(BF16)

    def b1(t, n):
        lo, hi = 256 * n, min(256 * n + 256, F)
        z = jnp.concatenate([z1b[t, c] for c in range(5)], axis=1)
        w1t = jnp.concatenate([w1s[c, lo:hi, :] for c in range(5)], axis=1)
        h = jax.lax.dot_general(z, w1t, (((1,), (1,)), ((), ())), preferred_element_type=F32)
        h = _gelu(h + b1f[:, lo:hi]).astype(BF16)
        for k in range(2):
            if lo + LANES * k < hi:
                n_col = min(LANES, hi - lo - LANES * k)
                hb[t % 2, 2 * n + k, :, :n_col] = h[:, LANES * k:LANES * k + n_col]

    def b2(t, c):
        h = jnp.concatenate([hb[t % 2, k] for k in range(13)] + [hb[t % 2, 13, :, :F - 13 * LANES]],
                            axis=1)
        val["y", t, c] = _dot(h, w2s[c]) + b2f[:, LANES * c:LANES * (c + 1)]

    def b_tail(t, layer):
        x2 = x1b[t] + jnp.concatenate([val.pop(("y", t, c)) for c in range(5)], axis=1)
        if layer == 1:
            for p, j in enumerate(JORD):
                outs[t, j] = x2[8 * p:8 * p + 8].astype(BF16)
            o_copy(t).start()
        else:
            for c, xc in enumerate(_tiles(x2)):
                x2s[t, c] = xc.astype(BF16)
            put_t(t, _layernorm(x2))

    t_copies[0].wait()
    x_copy(0).wait()
    ln0(0)
    for t in range(NT):
        if t == NT - 2:
            t_copies[1].wait()
            for c in w_copies[0]:
                c.wait()
        for g in range(3):
            c_mm(t, g)
        if t + 1 < NT:
            x_copy(t + 1).wait()
            ln0(t + 1)
        for g in range(3):
            c_fft(t, g)
            if t >= NT - 2:
                for q in range(16):
                    if q % 2 == t - (NT - 2) and q // 2 % 3 == g or (g == 2 and q // 2 >= 6 and q % 2 == t - (NT - 2) and q // 2 % 3 != 2):
                        pass
        if t >= NT - 2:
            for q in range(8):
                prep_w(0, 8 * (t - (NT - 2)) + q)
    for c in w_copies[1]:
        c.wait()
    for q in range(16):
        prep_w(1, q)
    for c in t_copies[2:]:
        c.wait()
    b1f[...] = b1s[...].astype(F32)[None, :]
    b2f[...] = b2s[...].astype(F32)[None, :]

    NH = NB // 2

    def spectral_middle(layer, c_last):
        if c_last:
            c_fft(NT - 1, 0)
        for b2_ in range(NH):
            p_fwd(b2_, 0)
        if c_last:
            c_fft(NT - 1, 1)
        for b2_ in range(NH):
            p_fwd(b2_, 1)
            p_inv(b2_, 0)
        if c_last:
            c_fft(NT - 1, 2)
        for b2_ in range(NH):
            p_fwd(b2_, 2)
            p_inv(b2_, 1)
        a_fft(0, 0)
        for b2_ in range(NH):
            p_inv(b2_, 2)
        a_mm(0, 0)
        a_fft(0, 1)
        a_mm(0, 1)
        a_fft(0, 2)
        a_mm(0, 2)
        a_tail(0, layer)

    def mlp_layer(layer):
        for i in range(NT):
            has_c = layer == 0 and i > 0
            has_a = i + 1 < NT
            b1(i, 0)
            if i > 0:
                b_tail(i - 1, layer)
            b1(i, 1)
            if has_c:
                c_mm(i - 1, 0)
            b1(i, 2)
            if has_c:
                c_fft(i - 1, 0)
                c_mm(i - 1, 1)
            b1(i, 3)
            if has_c:
                c_fft(i - 1, 1)
                c_mm(i - 1, 2)
            b1(i, 4)
            if has_c:
                c_fft(i - 1, 2)
            b1(i, 5)
            if has_a:
                a_fft(i + 1, 0)
            b1(i, 6)
            if has_a:
                a_mm(i + 1, 0)
                a_fft(i + 1, 1)
            b2(i, 0)
            if has_a:
                a_mm(i + 1, 1)
                a_fft(i + 1, 2)
            b2(i, 1)
            if has_a:
                a_mm(i + 1, 2)
            b2(i, 2)
            if has_a:
                a_tail(i + 1, layer)
            b2(i, 3)
            b2(i, 4)
        b_tail(NT - 1, layer)
        if layer == 0:
            for g in range(3):
                c_mm(NT - 1, g)

    spectral_middle(0, False)
    for c in w1_copies + w2_copies:
        c.wait()
    mlp_layer(0)
    spectral_middle(1, True)
    mlp_layer(1)
    for t in range(NT):
        o_copy(t).wait()


def _build(interpret=False):
    any_spec = pl.BlockSpec(memory_space=pltpu.HBM)
    scratch = [
        pltpu.VMEM((NT, NB, 8, D), BF16),
        pltpu.VMEM((NT, 5, R, LANES), BF16),
        pltpu.VMEM((NT, NB, 8, D), BF16),
        pltpu.VMEM((2, 16, NK, LANES), BF16),
        pltpu.VMEM((2, 3, 16 * PITCH, LANES), jnp.uint32),
        pltpu.VMEM((5, F, LANES), BF16),
        pltpu.VMEM((5, F, LANES), BF16),
        pltpu.VMEM((F,), BF16),
        pltpu.VMEM((D,), BF16),
        pltpu.VMEM((1, F), F32),
        pltpu.VMEM((1, D), F32),
        pltpu.VMEM((21, LANES, LANES), BF16),
        pltpu.VMEM((NB, 128, 128), BF16),
        pltpu.VMEM((NB, 128, 128), BF16),
        pltpu.VMEM((6, 8, LANES), jnp.int32),
        pltpu.VMEM((NB, 3, 128, LANES), BF16),
        pltpu.VMEM((NB, 3, 128, LANES), BF16),
        pltpu.VMEM((NB, 3, 128, LANES), BF16),
        pltpu.VMEM((NT, 5, R, LANES), BF16),
        pltpu.VMEM((NT, 5, R, LANES), BF16),
        pltpu.VMEM((NT, R, D), F32),
        pltpu.VMEM((2, 14, R, LANES), BF16),
        pltpu.SemaphoreType.DMA((N_SEM,)),
    ]
    return pl.pallas_call(
        _kernel,
        out_shape=jax.ShapeDtypeStruct((NB, NT, 8, D), BF16),
        in_specs=[any_spec] * 11,
        out_specs=any_spec,
        scratch_shapes=scratch,
        compiler_params=pltpu.CompilerParams(vmem_limit_bytes=100 * 1024 * 1024),
        interpret=interpret,
    )


def _run(A_x, A_w_r, A_w_i, B_w1, B_b1, B_w2, B_b2, interpret=False):
    bf = lambda a: jnp.asarray(a, dtype=BF16)
    out = _build(interpret)(
        A_x.reshape(NB, NT, 8, D), A_w_r.T, A_w_i.T, B_w1.T, B_b1, B_w2, B_b2,
        bf(_DM), bf(_MF), bf(_MI), jnp.asarray(_GT))
    return out.reshape(1, S, D)


@jax.jit
def pallas_interleave_layers__spectral_gfnet__dense_activation_gelu__prompt_kernel(
    A_x: jax.Array,
    A_w_r: jax.Array,
    A_w_i: jax.Array,
    B_x: jax.Array,
    B_w1: jax.Array,
    B_b1: jax.Array,
    B_w2: jax.Array,
    B_b2: jax.Array,
):
    del B_x
    return _run(A_x, A_w_r, A_w_i, B_w1, B_b1, B_w2, B_b2)
```

```python
import math

import jax
import jax.numpy as jnp
import numpy as np
import jax.experimental.pallas as pl
import jax.experimental.pallas.tpu as pltpu

S, D, F = 2048, 640, 1728
NK = D // 2 + 1
NB, NL = 32, 64
NT = 8
R = S // NT
LANES = 128
FM = F // LANES * LANES
EPS = 1e-5
JORD = [k + d for k in range(8) for d in (0, 16, 8, 24)]
JPOS = [JORD.index(j) for j in range(NB)]
F32, BF16, U32 = jnp.float32, jnp.bfloat16, jnp.uint32


W0 = 32


def _lane_layout():
    kd = -np.ones((3, LANES), np.int64)
    n = np.arange(64)
    for g, h, pair in ((0, 0, (1, 9)), (0, 1, (6, 4)), (1, 0, (2, 8)), (1, 1, (7, 3))):
        kd[g, 64 * h + n] = 10 * (n // 2) + np.array(pair)[n % 2]
    kd[2, W0 + n] = 5 * n
    kd[2, W0 + 64] = NK - 1
    assert sorted(kd[kd >= 0]) == list(range(NK))
    return kd


def _d_tables(kd):
    lp, ld, w = np.arange(64), np.arange(LANES), 2.0 / D
    fwd, inv = [], []
    for g in range(2):
        for k, is_v in ((kd[g, :64], False), (kd[g, 64:], True)):
            th = 2 * np.pi * np.outer(lp, k) / D
            c, s = np.cos(th), np.sin(th)
            sg = np.where(k % 5 == g + 1, 1.0, -1.0)[None, :]
            if not is_v:
                fwd.append(np.block([[c, -s], [sg * s, sg * c]]))
            else:
                fwd.append(np.block([[-s, c], [-sg * c, -sg * s]]))
            c, s, sg = c.T * w, s.T * w, sg.T
            if not is_v:
                inv.append(np.block([[c, sg * s], [-s, sg * c]]))
            else:
                inv.append(np.block([[-s, -sg * c], [c, -sg * s]]))
    th = 2 * np.pi * np.outer(ld, kd[2, W0:W0 + 64]) / D
    m0 = np.concatenate([np.cos(th), -np.sin(th)], axis=1)
    m0[:, 64] = (-1.0) ** ld
    n0 = np.concatenate([np.cos(th).T * w, -np.sin(th).T * w], axis=0)
    n0[0], n0[64] = 1.0 / D, (-1.0) ** ld / D
    m0, n0 = np.roll(m0, W0, axis=1), np.roll(n0, W0, axis=0)
    return np.stack(fwd + [m0]), np.stack(inv + [n0]) / S


def _s_tables():
    a = np.arange(NL)[:, None]
    l = np.arange(NL)[None, :]
    kap = 16 * (np.arange(NL) // 8) + np.arange(NL) % 8
    mf = np.zeros((NB, 128, 128))
    for b in range(NB):
        m = np.exp(-2j * np.pi * l * (NB * a + b) / S)
        mf[b][np.ix_(kap, kap)] = m.real
        mf[b][np.ix_(kap, kap + 8)] = -m.imag
        mf[b][np.ix_(kap + 8, kap)] = m.imag
        mf[b][np.ix_(kap + 8, kap + 8)] = m.real
    return mf


_KD = _lane_layout()
_DF, _DI = _d_tables(_KD)


def _d_direct(kd):
    ld, out = np.arange(LANES), []
    for g in range(3):
        used = kd[g] >= 0
        th = 2 * np.pi * np.outer(ld, np.where(used, kd[g], 0)) / D
        out += [np.cos(th) * used, -np.sin(th) * used]
        assert g == 2 or ((kd[g] % 5 == g + 1) == (ld % 2 == 0)).all()
    return np.stack(out)


_DD = _d_direct(_KD)
_MF = _s_tables()

C1, S1 = math.cos(2 * math.pi / 5), math.sin(2 * math.pi / 5)
C2, S2 = math.cos(4 * math.pi / 5), math.sin(4 * math.pi / 5)


def _fft(xr, xi, sign):
    n = len(xr)
    if n == 1:
        return list(xr), list(xi)
    if n == 2:
        return [xr[0] + xr[1], xr[0] - xr[1]], [xi[0] + xi[1], xi[0] - xi[1]]
    ur, ui = _fft(xr[0::2], xi[0::2], sign)
    zr, zi = _fft(xr[1::4], xi[1::4], sign)
    wr, wi = _fft(xr[3::4], xi[3::4], sign)
    q = n // 4
    outr, outi = [None] * n, [None] * n

    def twiddle(r, i, k):
        k %= n
        if k == 0:
            return r, i
        if 8 * k == n:
            h = math.sqrt(0.5)
            return ((r - i) * h, (r + i) * h) if sign > 0 else ((r + i) * h, (i - r) * h)
        if 8 * k == 3 * n:
            h = math.sqrt(0.5)
            return ((r + i) * -h, (r - i) * h) if sign > 0 else ((i - r) * h, (r + i) * -h)
        c, s = math.cos(2 * math.pi * k / n), sign * math.sin(2 * math.pi * k / n)
        return r * c - i * s, r * s + i * c

    for k in range(q):
        ar, ai = twiddle(zr[k], zi[k], k)
        br, bi = twiddle(wr[k], wi[k], 3 * k)
        sr, si, dr, di = ar + br, ai + bi, ar - br, ai - bi
        outr[k], outi[k] = ur[k] + sr, ui[k] + si
        outr[k + 2 * q], outi[k + 2 * q] = ur[k] - sr, ui[k] - si
        if sign > 0:
            outr[k + q], outi[k + q] = ur[k + q] - di, ui[k + q] + dr
            outr[k + 3 * q], outi[k + 3 * q] = ur[k + q] + di, ui[k + q] - dr
        else:
            outr[k + q], outi[k + q] = ur[k + q] + di, ui[k + q] - dr
            outr[k + 3 * q], outi[k + 3 * q] = ur[k + q] - di, ui[k + q] + dr
    return outr, outi


def _twiddle32(r, i, k, sign):
    k %= 32
    h = math.sqrt(0.5)
    if k == 0:
        return r, i
    if k == 8:
        return (-i, r) if sign > 0 else (i, -r)
    if k == 4:
        return ((r - i) * h, (r + i) * h) if sign > 0 else ((r + i) * h, (i - r) * h)
    if k == 12:
        return ((r + i) * -h, (r - i) * h) if sign > 0 else ((i - r) * h, (r + i) * -h)
    c, s = math.cos(2 * math.pi * k / 32), sign * math.sin(2 * math.pi * k / 32)
    return r * c - i * s, r * s + i * c


def _dft4(xr, xi, sign):
    ar, ai, br, bi = xr[0] + xr[2], xi[0] + xi[2], xr[0] - xr[2], xi[0] - xi[2]
    cr, ci, dr, di = xr[1] + xr[3], xi[1] + xi[3], xr[1] - xr[3], xi[1] - xi[3]
    if sign > 0:
        return [ar + cr, br - di, ar - cr, br + di], [ai + ci, bi + dr, ai - ci, bi - dr]
    return [ar + cr, br + di, ar - cr, br - di], [ai + ci, bi - dr, ai - ci, bi + dr]


def _tiles(x):
    return [x[:, LANES * c:LANES * (c + 1)] for c in range(x.shape[1] // LANES)]


def _layernorm(x):
    m = jnp.mean(x, axis=-1, keepdims=True)
    xc = x - m
    v = jnp.mean(xc * xc, axis=-1, keepdims=True)
    return xc * jax.lax.rsqrt(v + EPS)


def _lane(shape):
    return jax.lax.broadcasted_iota(jnp.int32, shape, 1)


def _swap(x):
    return pltpu.roll(x, LANES // 2, axis=1)


def _half_twiddle(b, lo):
    return (jnp.where(lo, 1.0, math.cos(2 * math.pi * b / 10)),
            jnp.where(lo, 0.0, -math.sin(2 * math.pi * b / 10)))


def _d_split(z, halves=True):
    z0, z1, z2, z3, z4 = _tiles(z)
    lo = _lane(z0.shape) < 64
    a, b, c, e = z1 + z4, z2 + z3, z1 - z4, z2 - z3
    p = a + b
    base = z0 + p * -0.25
    m2 = (a - b) * (math.sqrt(5.0) / 4)
    out = []
    for g, (tr, ti) in enumerate(((base + m2, c * -S1 + e * -S2), (base - m2, e * S1 - c * S2))):
        if not halves:
            out += [tr, ti]
            continue
        cw, sw = _half_twiddle(g + 1, lo)
        tr, ti = tr * cw - ti * sw, tr * sw + ti * cw
        pp, qq = jnp.where(lo, tr, ti), _swap(jnp.where(lo, ti, tr))
        out += [pp + qq, pp - qq]
    return out + [z0 + p]


def _d_merge(u1, v1, u2, v2, s0):
    lo = _lane(s0.shape) < 64
    sig = []
    for g, (u, v) in enumerate(((u1, v1), (u2, v2))):
        pp, qq = u + v, _swap(u - v)
        tr, ti = jnp.where(lo, pp, qq), jnp.where(lo, qq, pp)
        cw, sw = _half_twiddle(g + 1, lo)
        sig += [tr * cw + ti * sw, ti * cw - tr * sw]
    a1, b1, a2, b2 = sig
    p = a1 + a2
    base = s0 + p * -0.25
    m2 = (a1 - a2) * (math.sqrt(5.0) / 4)
    e1, e2 = base + m2, base - m2
    o1 = b1 * S1 + b2 * S2
    o2 = b1 * S2 - b2 * S1
    return jnp.concatenate([s0 + p, e1 - o1, e2 - o2, e2 + o2, e1 + o1], axis=1)


def _gelu(h):
    c = math.sqrt(2.0 / math.pi)
    u = h * (c + (c * 0.044715) * (h * h))
    hh = 0.5 * h
    return hh + hh * jnp.tanh(u)


def _dot(a, b):
    return jnp.dot(a, b, preferred_element_type=F32)


PW = (0, 0, 2, 2, 2, 2, 2, 2, 8, 7, 5)
W_STEP = [r for r, n in enumerate(PW) for _ in range(n)]
WAITS = (["x%d" % r for r in range(len(PW))]
         + ["Wa", "Wb", "Wc", "W1", "W2", "out"])
PITCH = NL + 1


_REGIONS = dict(
    tokf=("F", 1, 8), tokl=("L", 1, 8),
    cst=("F", 2 * 3 * 4, 128),
    ast=("F", 3 * 4, 128),
    ub=("F", NB * 3, 64),
    vb=("F", NT * 3 * 4, 64),
    ab=("F", 5, 128),
    sb=("L", 8, 160),
    x1b=("L", NT * 5, 256),
    z1b=("L", NT * 5, 128),
    x2f=("L", 2 * 8, 160),
    xr=("L", NT * 8, 80),
    tb=("L", NT * 5, 128),
    hb=("H", 2 * 14, 128),
    b1c=("H", 1, 64),
)
_OFFSET, ARENA_WORDS = {}, {"F": 0, "L": 0, "H": 0}
for _name, (_arena, _tiles_, _rows) in _REGIONS.items():
    _OFFSET[_name] = ARENA_WORDS[_arena]
    ARENA_WORDS[_arena] += _tiles_ * _rows


class _Packed:
    def __init__(self, ref):
        self.ref, self.words = ref, ref.bitcast(U32)

    def __setitem__(self, key, val):
        self.ref[key] = val.astype(BF16)

    def __getitem__(self, key):
        return self.get(key)

    def get(self, key, tok=None):
        *lead, rs, cs = key
        w = self.words[(*lead, slice(rs.start // 2, rs.stop // 2), cs)]
        if tok is not None:
            w = jnp.concatenate([w[:8] | tok, w[8:]], axis=0)
        return pltpu.bitcast(w, BF16)


class _Region:
    def __init__(self, arenas, zero, name):
        arena, _, self.rows = _REGIONS[name]
        self.buf, self.off, self.zero = arenas[arena], _OFFSET[name], zero

    def store(self, tile, row, val):
        at = self.off + tile * self.rows + row
        if val.dtype == F32:
            self.buf.words[at:at + val.shape[0], :] = pltpu.bitcast(val, U32)
        else:
            self.buf.ref[2 * at:2 * at + val.shape[0], :] = val

    def load(self, tile, dtype, row=0, n=None, serial=False, tok=None):
        at, n = self.off + tile * self.rows + row, self.rows if n is None else n
        rs = pl.ds(pl.multiple_of(self.zero + at, 8), n) if serial else slice(at, at + n)
        w = self.buf.words[rs, :]
        if tok is not None:
            w = jnp.concatenate([w[:8] | tok, w[8:]], axis=0)
        return pltpu.bitcast(w, dtype)


def _kernel(x_hbm, wr_hbm, wi_hbm, w1_hbm, b1_hbm, w2_hbm, b2_hbm,
            df_hbm, di_hbm, mf_hbm, dd_hbm,
            out_hbm, *scratch):
    (xs, out_a, out_b, wsr, wp, w1r, w2r, b1s, b2s, dfr, dir_, mfr, mir, wn, ddr,
     yr_, arena_f, arena_l, arena_h, zsem, bsem, sems) = scratch
    w1s, w2s, dfs, dis, mfs, mis, yb = [
        _Packed(r) for r in (w1r, w2r, dfr, dir_, mfr, mir, yr_)]
    zero = pl.semaphore_read(zsem)
    arenas = {"F": _Packed(arena_f), "L": _Packed(arena_l), "H": _Packed(arena_h)}
    (tokf, tokl, cst, ast, ub, vb, ab, sb, x1b, z1b, x2f, xr, tb, hb, b1c) = [
        _Region(arenas, zero, n) for n in _REGIONS]
    ALL = FULL = slice(0, LANES)
    outs = (out_a, out_b)
    dds = _Packed(ddr)

    groups = {name: [] for name in WAITS}

    def copy(name, src, dst):
        groups[name].append(pltpu.make_async_copy(src, dst, sems.at[WAITS.index(name)]))
        groups[name][-1].start()

    def wait(name):
        for c in groups.pop(name):
            c.wait()

    def copy_w(i):
        (a, q), name = divmod(i, 16), "x%d" % W_STEP[i]
        w_hbm = (wr_hbm, wi_hbm)[a]
        if q == 0:
            copy(name, w_hbm.at[NK - 1:NK, :], wn.at[a])
        copy(name, w_hbm.at[:NK - 1, LANES * q:LANES * (q + 1)], wsr.at[a, q])

    def copy_out(t, h):
        copy("out", outs[h].at[t], out_hbm.at[:, 4 * h:4 * h + 4, t])

    copy("x0", x_hbm.at[:, 0], xs.at[0])
    for g in range(3):
        copy("x1", dd_hbm.at[2 * g:2 * g + 2], ddr.at[4 * g:4 * g + 2])
    copy("x1", x_hbm.at[:, 1], xs.at[1])
    for t in range(2, NT):
        copy_w(2 * t - 4)
        copy_w(2 * t - 3)
        copy("x%d" % t, x_hbm.at[:, t], xs.at[t])
    for i in range(2 * NT - 4, 32):
        copy_w(i)
    copy("Wa", mf_hbm.at[:NB // 4], mfr.at[:NB // 4])
    copy("Wb", mf_hbm.at[NB // 4:NB // 2], mfr.at[NB // 4:NB // 2])
    copy("Wb", di_hbm, dir_)
    copy("Wc", mf_hbm.at[NB // 2:], mfr.at[NB // 2:])
    for name, b_hbm, b_vmem, w_hbm, w_vmem in (("W1", b1_hbm, b1s, w1_hbm, w1r),
                                               ("W2", b2_hbm, b2s, w2_hbm, w2r)):
        copy(name, b_hbm, b_vmem)
        for c in range(5):
            copy(name, w_hbm.at[:, LANES * c:LANES * (c + 1)], w_vmem.at[c])
    copy("W2", df_hbm, dfr)

    def rows(e):
        return slice(32 * e, 32 * e + 32)

    for r in (tokf, tokl):
        r.store(0, 0, jnp.zeros((8, LANES), F32))
    wp[6, 0:8, :] = jnp.zeros((8, LANES), U32)

    def token():
        v = (tokf.load(0, U32, serial=True) | tokl.load(0, U32, serial=True)
             | wp[6, pl.ds(pl.multiple_of(zero, 8), 8), :])
        return v & zero.astype(U32)

    toks = [None]
    pending = []

    def fence(lag=2):
        pending.append(token())
        if len(pending) > lag:
            toks[0] = pending[-1 - lag]

    def barrier():
        pl.semaphore_signal(bsem, 1)
        pl.semaphore_wait(bsem, 1)

    def put_t(t, e, z, halves=True):
        for c, v in enumerate(_d_split(z, halves)):
            tb.store(5 * t + c, 16 * e, v.astype(BF16))

    zeros = [zero, zero * 2, zero * 3]

    def ln0(t, e):
        def load(i):
            return jnp.concatenate([xs[t, j + zeros[i]].astype(F32)
                                    for j in JORD[4 * e:4 * e + 4]], axis=0)
        xr.store(8 * t + e, 0, jnp.concatenate(_tiles(load(0)), axis=0).astype(BF16))
        put_t(t, e, _layernorm(load(0)), halves=False)

    def part(h):
        return (range(4), range(4, 8), range(4, 6), range(6, 8))[h]

    def c1(t, g, h, direct=False):
        lane, es = _lane((8, LANES)), part(h)
        at = (16 * es[0], 16 * len(es))
        if direct:
            cs = (2 * g, 2 * g + 1) if g < 2 else (4,)
            lhs = jnp.concatenate([tb.load(5 * t + c, BF16, *at) for c in cs], axis=1)
            rhs = jnp.concatenate([jnp.concatenate(
                [dds.get((4 * g + 2 * i + j, FULL, ALL), toks[0] if i + j == 0 else None)
                 for j in range(2)], axis=1) for i in range(len(cs))], axis=0)
            ri = _dot(lhs, rhs)
        else:
            u, v = [_dot(tb.load(5 * t + c, BF16, *at), dfs.get((c, FULL, ALL), toks[0]))
                    for c in ((2 * g, 2 * g + 1) if g < 2 else (4, 4))]
        for k in es:
            xr, xi = [], []
            for r in range(4):
                p = 8 * JPOS[k + 8 * r] - 32 * es[0]
                if direct:
                    xr.append(ri[p:p + 8, :LANES])
                    xi.append(ri[p:p + 8, LANES:])
                elif g < 2:
                    uu, vv = u[p:p + 8], v[p:p + 8]
                    xr.append(jnp.where(lane < 64, uu, vv))
                    xi.append(_swap(jnp.where(lane < 64, vv, uu)))
                else:
                    uu = u[p:p + 8]
                    xr.append(jnp.where((lane >= W0) & (lane <= W0 + 64), uu, 0.0))
                    xi.append(jnp.where((lane > W0) & (lane < W0 + 64), _swap(uu), 0.0))
            yr, yi = _dft4(xr, xi, -1)
            for m in range(4):
                wr_, wi_ = _twiddle32(yr[m], yi[m], k * m, -1)
                cst.store(12 * (t % 2) + 4 * g + m, 16 * k, jnp.concatenate([wr_, wi_], axis=0))

    def c2(t, g):
        for m in range(4):
            x = cst.load(12 * (t % 2) + 4 * g + m, F32, serial=m == 0)
            ur, ui = _fft([x[16 * k:16 * k + 8] for k in range(8)],
                          [x[16 * k + 8:16 * k + 16] for k in range(8)], -1)
            for q in range(8):
                ub.store(3 * (m + 4 * q) + g, 8 * t,
                         jnp.concatenate([ur[q], ui[q]], axis=0).astype(BF16))

    def prep_w(a, q):
        lo, hi = jnp.uint32(0x0000FFFF), jnp.uint32(0xFFFF0000)
        w = [[wsr.bitcast(U32)[a, q, pl.ds(rho + 40 * j, 8, stride=5), :] for j in range(4)]
             for rho in range(5)]
        nyq = pltpu.bitcast(wn[a, :, LANES * q:LANES * (q + 1)].astype(F32), U32) >> 16
        nyq = jnp.where(jax.lax.broadcasted_iota(jnp.int32, (16, LANES), 0) == 0, nyq, 0)
        groups = [
            [(w[0][j] >> 16) | (w[4][j] & hi) for j in range(4)]
            + [(w[3][j] & lo) | (w[2][j] << 16) for j in range(4)],
            [(w[1][j] & lo) | (w[4][j] << 16) for j in range(4)]
            + [(w[3][j] >> 16) | (w[1][j] & hi) for j in range(4)],
            [jnp.zeros((W0 // 2, LANES), U32)] + [(w[0][j] & lo) | (w[2][j] & hi) for j in range(4)]
            + [nyq]]
        for g, rows_ in enumerate(groups):
            word = pltpu.bitcast(pltpu.bitcast(jnp.concatenate(rows_, axis=0), BF16).T, U32)
            for r in range(8):
                wp[3 * a + g, pl.ds(PITCH * 8 * (r % 2) + 4 * q + r // 2, 8, stride=PITCH), :] = (
                    word[8 * r:8 * r + 8])

    def p_fwd(b2_, g):
        wg = [wp[3 * a + g, pl.ds(PITCH * b2_, NL), :] for a in range(2)]
        for par in range(2):
            b = 2 * b2_ + par
            xf = _dot(mfs.get((b, FULL, ALL), toks[0]), ub.load(3 * b + g, BF16))
            ys = []
            for i in range(8):
                wr, wi = [pltpu.bitcast(w[8 * i:8 * i + 8] << 16 if par == 0 else
                                        w[8 * i:8 * i + 8] & jnp.uint32(0xFFFF0000), F32) for w in wg]
                xr, xi = xf[16 * i:16 * i + 8], xf[16 * i + 8:16 * i + 16]
                ys += [xr * wr - xi * wi, xr * wi + xi * wr]
            yb[b, g, FULL, ALL] = jnp.concatenate(ys, axis=0)

    def p_inv(b2_, g, h):
        for b in (2 * b2_, 2 * b2_ + 1):
            v = _dot(mis.get((b, slice(64 * h, 64 * h + 64), ALL), toks[0]), yb[b, g, FULL, ALL])
            for t in range(4):
                vb.store(12 * (4 * h + t) + 4 * g + b % 4, 8 * (b // 4),
                         v[16 * t:16 * t + 16].astype(BF16))

    def a1(t, g):
        for m in range(4):
            v = vb.load(12 * t + 4 * g + m, BF16, serial=m == 0).astype(F32)
            zr, zi = _fft([v[16 * q:16 * q + 8] for q in range(8)],
                          [v[16 * q + 8:16 * q + 16] for q in range(8)], +1)
            for k in range(8):
                wr_, wi_ = _twiddle32(zr[k], zi[k], k * m, +1)
                ast.store(4 * g + k // 2, 64 * (k % 2) + 16 * m, jnp.concatenate([wr_, wi_], axis=0))

    def a2(t, g, h):
        lane = _lane((8, LANES))
        for k2 in (2 * h, 2 * h + 1):
            x = ast.load(4 * g + k2, F32, serial=k2 == 0)
            us, vs = [], []
            for kk in range(2):
                yr, yi = _dft4([x[64 * kk + 16 * m:64 * kk + 16 * m + 8] for m in range(4)],
                               [x[64 * kk + 16 * m + 8:64 * kk + 16 * m + 16] for m in range(4)], +1)
                for r in (0, 2, 1, 3):
                    rr, ri = yr[r], _swap(yi[r])
                    if g < 2:
                        us.append(jnp.where(lane < 64, rr, ri))
                        vs.append(jnp.where(lane < 64, ri, rr))
                    else:
                        us.append(jnp.where((lane >= W0) & (lane <= W0 + 64), rr, ri))
            ab.store(2 * g, 32 * k2, jnp.concatenate(us, axis=0).astype(BF16))
            if g < 2:
                ab.store(2 * g + 1, 32 * k2, jnp.concatenate(vs, axis=0).astype(BF16))

    def a3(t, g, h):
        for c in ((2 * g, 2 * g + 1) if g < 2 else (4,)):
            s_ = _dot(ab.load(c, BF16, 64 * h, 64), dis.get((c, FULL, ALL), toks[0]))
            for e in range(4):
                sb.store(4 * h + e, 32 * c, s_[rows(e)])

    def a4(t, e):
        s_ = sb.load(e, F32, serial=e % 4 == 0)
        y = _d_merge(*[s_[rows(c)] for c in range(5)])
        x = xr.load(8 * t + e, BF16).astype(F32)
        x1 = jnp.concatenate([x[rows(c)] for c in range(5)], axis=1) + y
        for c, xc in enumerate(_tiles(x1)):
            x1b.store(5 * t + c, 32 * e, xc)
        for c, zc in enumerate(_tiles(_layernorm(x1))):
            z1b.store(5 * t + c, 16 * e, zc.astype(BF16))

    nt_dims = (((1,), (1,)), ((), ()))

    def b1(t, n, h):
        lo, hi = 256 * n, min(256 * n + 256, FM)
        w1t = jnp.concatenate([w1s.get((c, slice(lo, hi), ALL), toks[0] if c == 0 else None)
                               for c in range(5)], axis=1)
        z = jnp.concatenate([z1b.load(5 * t + c, BF16, 64 * h, 64) for c in range(5)], axis=1)
        y = jax.lax.dot_general(z, w1t, nt_dims, preferred_element_type=F32)
        y = _gelu(y + b1s[lo:hi].astype(F32)[None, :]).astype(BF16)
        for k, yk in enumerate(_tiles(y)):
            hb.store(14 * (t % 2) + 2 * n + k, 64 * h, yk)

    def br(t):
        w1t = jnp.concatenate([w1s[c, FM:F, ALL] for c in range(5)], axis=1)
        ys = []
        for h in range(2):
            z = jnp.concatenate([z1b.load(5 * t + c, BF16, 64 * h, 64, tok=toks[0] if c == 0 else None)
                                 for c in range(5)], axis=1)
            y = jax.lax.dot_general(w1t, z, nt_dims, preferred_element_type=F32)
            ys.append(_gelu(y + b1c.load(0, F32)).astype(BF16))
        hb.store(14 * (t % 2) + 13, 0, jnp.concatenate(ys, axis=0).T)

    def prep_b1():
        v = b1s[FM - LANES:F].astype(F32)[None, :][:, LANES:]
        eye = [jax.lax.broadcasted_iota(jnp.int32, (F - FM, F - FM), d) for d in range(2)]
        col = jnp.sum(jnp.where(eye[0] == eye[1], v, 0.0), axis=1, keepdims=True)
        b1c.store(0, 0, jnp.broadcast_to(col, (F - FM, LANES)))

    def b2(t, c, h, layer):
        cols, es = slice(LANES * c, LANES * (c + 1)), part(h)
        y = jnp.concatenate([hb.load(14 * (t % 2) + k, BF16, 16 * es[0] % (R // 2 if k < 13 else 64),
                                     16 * len(es)) for k in range(14)], axis=1)
        rest = [w2s[c, FM:F, ALL], jnp.zeros((F - FM, LANES), BF16)]
        w = jnp.concatenate([w2s.get((c, slice(0, FM), ALL), toks[0])] + rest[::-1 if h else 1], axis=0)
        y = _dot(y, w) + b2s[cols].astype(F32)[None, :]
        x2 = x1b.load(5 * t + c, F32, 32 * es[0], 32 * len(es)) + y
        for i, e in enumerate(es):
            if layer == 0:
                x2f.store(8 * (t % 2) + e, 32 * c, x2[rows(i)])
            else:
                for p in range(4):
                    outs[e // 4][t, JORD[p] // 8, e % 4, :, cols] = x2[rows(i)][8 * p:8 * p + 8].astype(BF16)

    def b3(t, e):
        x2 = x2f.load(8 * (t % 2) + e, F32, serial=e % 4 == 0)
        xr.store(8 * t + e, 0, x2.astype(BF16))
        put_t(t, e, _layernorm(jnp.concatenate([x2[rows(c)] for c in range(5)], axis=1)))

    def slot(layer, i, order):
        for tok in order.split():
            k = tok[:2]
            if tok[0] == "@":
                layer, i = map(int, tok[1:].split("."))
            elif tok in WAITS:
                wait(tok)
            elif k in ("pf", "pi"):
                for b2_ in range(4 * int(tok[3]), 4 * int(tok[3]) + 4):
                    if k == "pf":
                        p_fwd(b2_, int(tok[2]))
                    else:
                        p_inv(b2_, int(tok[2]), "ab".index(tok[4]))
            elif k == "tr":
                for b in range(8 * int(tok[2]), 8 * int(tok[2]) + 8):
                    mis[b, FULL, ALL] = mfs[b, FULL, ALL].T
            elif k == "od":
                for h in range(2):
                    for t in range(i):
                        copy_out(t, h)
            elif k == "OD":
                copy_out(i, "ab".index(tok[2]))
            elif len(tok) == 2:
                {"ff": fence, "BB": barrier, "pb": prep_b1, "br": lambda: br(i)}[k]()
            else:
                args = [int(tok[2])] + ["abcd".index(h) for h in tok[3:]] + [layer] * (k == "b2")
                task, dt = {"b1": (b1, 0), "b2": (b2, 0), "b3": (b3, -1), "c1": (c1, -1),
                            "c2": (c2, -1), "B3": (b3, 0), "C1": (c1, 0), "C2": (c2, 0),
                            "a1": (a1, 1), "a2": (a2, 1), "a3": (a3, 1), "a4": (a4, 1)}[k]
                task(i + dt, *args)

    def head(r):
        wait("x%d" % r)
        if r == 1:
            odd = _lane((64, LANES)) % 2 == 1
            for k in (0, 1, 4, 5):
                dds.words[k + 3 - 2 * (k % 2)] = dds.words[k] ^ jnp.where(
                    odd if k % 2 == 0 else ~odd, jnp.uint32(0x80008000), jnp.uint32(0))
        pw = [divmod(i, 16) for i in range(32) if W_STEP[i] == r]
        for tok in "l7 d0 l5 l1 d2 c00 c01 c10 c11 d1 l3 l4 l6 c21 c20 f f w1 l0 l2 w1 w1 w16".split():
            if tok[0] == "l" and r < NT:
                ln0(r, int(tok[1]))
            elif tok[0] == "c" and 0 <= r - 1 < NT:
                c1(r - 1, int(tok[1]), int(tok[2]), True)
            elif tok[0] == "d" and 0 <= r - 2 < NT:
                c2(r - 2, int(tok[1]))
            elif tok[0] == "f":
                fence(1)
            elif tok[0] == "w":
                n = int(tok[1:])
                for a_, q in pw[:n]:
                    prep_w(a_, q)
                pw = pw[n:]

    ORD1 = ("ff b10a b30 a10 b31 b32 b10b ff b11a b11b ff b12a b33 a11 b34 b12b b13a a12 ff b13b "
            "b14a a20a b35 a20b b14b c10a a21a b36 ff b15a b37 c10b ff b15b c12b a22a a22b b16a "
            "ff br a30a a21b ff b16b c20 a32b ff b20a c11b c11a c21 b20b c12a a30b a31a b21a a32a "
            "ff b21b b22a a41 a40 c22 b22b a42 a31b a47 a43 a45 ff b23a a46 ff b23b a44 ff b24a "
            "ff b24b")
    ORD2 = ("ff b10a ff b10b a12 a11 a10 b11a ff b11b ff b12a a20a b12b b13a b13b a20b a22a b14a "
            "a30a a21b b14b ff b15a a21a a32a b15b b16a a22b br b16b a32b ff b20a a30b a31b a45 "
            "ff b20b b21a a31a a41 a43 b21b b22a ff b22b a42 a40 ff b23a a44 a47 ff b23b b24a "
            "b24b a46")
    LAST2 = ("ff b10a ff b10b od b11a b11b b12a b12b ff b13a b13b ff b14a b14b ff b15a b15b b16a "
             "br b16b ff b20a b21a b22a b23a b24a ff b20b ODa b21b ff b22b b23b ff b24b")
    JOIN0 = ("Wa pf00 pf20 pf10 ff Wb pf01 tr1 tr0 pf11 pf21 Wc tr2 pf13 pf03 pf02 pf12 tr3 pf22 "
             "pi00a pf23 ff pi03a pi01a pi12a pi10a pi02a pi11a @0.-1 a10 pi13a a11 pi21a pi23a "
             "a20a pi20a pi22a a21a pi02b a12 pi00b a22a pi03b a20b a30a pi11b a31a pi01b a32a "
             "pi20b a41 pi10b a43 a21b a40 pi12b a42 a31b pi22b pi23b pi13b a30b pi21b a22b a32b "
             "BB W1 pb @0.0 b10a @0.-1 a45 @0.0 b11a @0.-1 a46 a44 @0.0 a10 ff b12a ff b13a @0.-1 "
             "a47 @0.0 a20a a11 b14a a12 ff a22a b15a a21a b16a b10b b11b b12b b13b a20b a22b "
             "a21b ff ff b14b ff b15b b16b br a30a a32a a30b a31a W2 b20a ff b20b a40 b21a b21b "
             "a31b a32b b22a b22b a43 a46 b23a b23b a44 a42 b24a a45 b24b a47 a41")
    MID = ("b10a b10b ff b30 b31 b11a b11b ff b12a b12b b33 ff ff ff b34 b32 b13a b13b b35 b36 "
           "b37 ff b14a ff b14b c10b b15a c11a c10a b15b ff c20 c11b c12b ff c21 b16a br b16b ff "
           "c12a b20a c22 b21a ff b22a b23a b24a ff ff B31 B30 B33 b20c b21c b22c b23c B32 ff "
           "b24c C10a C11a B34 b20d C12a b21d ff ff b22d B35 ff C11c b23d C10c b24d C12c B36 B37 "
           "ff C10d C20 C11d C12d pf00 pf01 C22 pf03 C21 pf10 pf11 pf02 pf23 pf20 pf21 pf12 pf13 "
           "pf22 pi01a pi02a pi03a pi00a pi12a pi11a @1.-1 a10 pi10a pi13a a11 ff a20a pi21a "
           "pi22a pi23a pi20a a21a pi00b a12 pi01b a22a pi03b a20b ff pi10b pi02b a30a a31a ff "
           "a32a a40 pi11b a41 pi13b pi12b a42 pi20b ff a22b a21b pi21b a43 pi22b pi23b a30b a31b "
           "a32b @1.0 b10a ff b11a @1.-1 a46 a45 a44 @1.0 a10 ff @1.-1 a47 @1.0 b12a ff b13a a11 "
           "ff b14a b15a a12 b16a a20a a22a b10b b11b a20b a21b b12b ff a21a b13b a22b b14b a30a "
           "ff b15b b16b br a32a a31a a30b b20a ff ff b20b a40 b21a b21b a32b a31b a41 b22a a43 "
           "a42 b22b a46 b23a b23b a44 a45 ff b24a a47 b24b")

    for r in range(len(PW)):
        head(r)
    slot(0, 0, JOIN0)
    for i in range(1, NT - 1):
        slot(0, i, ORD1)
    slot(0, NT - 1, MID)
    for i in range(1, NT - 1):
        slot(1, i, ORD2)
    slot(1, NT - 1, LAST2 + " ODb out")
    assert not groups


def _build():
    any_spec = pl.BlockSpec(memory_space=pltpu.HBM)
    scratch = [
        pltpu.VMEM((NT, NB, 8, D), BF16),
        pltpu.VMEM((NT, 4, 4, 8, D), BF16),
        pltpu.VMEM((NT, 4, 4, 8, D), BF16),
        pltpu.VMEM((2, 16, NK - 1, LANES), BF16),
        pltpu.VMEM((7, 16 * PITCH, LANES), U32),
        pltpu.VMEM((5, F, LANES), BF16),
        pltpu.VMEM((5, F, LANES), BF16),
        pltpu.VMEM((F,), BF16),
        pltpu.VMEM((D,), BF16),
        pltpu.VMEM((5, LANES, LANES), BF16),
        pltpu.VMEM((5, LANES, LANES), BF16),
        pltpu.VMEM((NB, 128, LANES), BF16),
        pltpu.VMEM((NB, 128, LANES), BF16),
        pltpu.VMEM((2, 1, S), BF16),
        pltpu.VMEM((10, LANES, LANES), BF16),
        pltpu.VMEM((NB, 3, 128, LANES), BF16),
        pltpu.VMEM((2 * ARENA_WORDS["F"], LANES), BF16),
        pltpu.VMEM((2 * ARENA_WORDS["L"], LANES), BF16),
        pltpu.VMEM((2 * ARENA_WORDS["H"], LANES), BF16),
        pltpu.SemaphoreType.REGULAR,
        pltpu.SemaphoreType.REGULAR,
        pltpu.SemaphoreType.DMA((len(WAITS),)),
    ]
    return pl.pallas_call(
        _kernel,
        out_shape=jax.ShapeDtypeStruct((4, 8, NT, 8, D), BF16),
        in_specs=[any_spec] * 11,
        out_specs=any_spec,
        scratch_shapes=scratch,
        compiler_params=pltpu.CompilerParams(vmem_limit_bytes=100 * 1024 * 1024),
    )


@jax.jit
def pallas_interleave_layers__spectral_gfnet__dense_activation_gelu__prompt_kernel(
    A_x: jax.Array,
    A_w_r: jax.Array,
    A_w_i: jax.Array,
    B_x: jax.Array,
    B_w1: jax.Array,
    B_b1: jax.Array,
    B_w2: jax.Array,
    B_b2: jax.Array,
):
    del B_x
    out = _build()(
        A_x.reshape(NB, NT, 8, D), A_w_r.T, A_w_i.T, B_w1.T, B_b1, B_w2, B_b2,
        *[m.astype(jnp.bfloat16) for m in (_DF, _DI, _MF, _DD)])
    return out.reshape(1, S, D)
```
